```python
import os as _os
_os.environ.setdefault("JAX_PLATFORMS", "cpu")
import jax
import jax.numpy as jnp

def _softmax(x, axis=-1):
    return jax.nn.softmax(x, axis=axis)
def _gelu(x):
    return jax.nn.gelu(x, approximate=True)
def _silu(x):
    return jax.nn.silu(x)
def _sigmoid(x):
    return jax.nn.sigmoid(x)
def _layernorm(x, axis=-1, eps=1e-5):
    m = jnp.mean(x, axis=axis, keepdims=True)
    v = jnp.var(x, axis=axis, keepdims=True)
    return (x - m) / jnp.sqrt(v + eps)
def _scatter_add(tgt, idx, src, axis=0):
    return tgt.at[idx].add(src)
def _segment_sum(src, seg, n):
    return jax.ops.segment_sum(src, seg, n)
class _Rng:
    def __init__(self, key):
        self._k = key
    def _next(self):
        self._k, sub = jax.random.split(self._k)
        return sub
    def normal(self, shape):
        return jax.random.normal(self._next(), shape, dtype=jnp.bfloat16)
    def randint(self, lo, hi, shape):
        return jax.random.randint(self._next(), shape, lo, hi, dtype=jnp.int32)
    def uniform(self, shape, lo=0.0, hi=1.0):
        return jax.random.uniform(self._next(), shape, jnp.bfloat16, lo, hi)
    def permutation(self, n):
        return jax.random.permutation(self._next(), n)


kernel_name = 'standalone__linear_kernel_hedgehog__prompt'

def setup_inputs():
    _rng = _Rng(jax.random.key(int.from_bytes(__import__("os").urandom(4), "little")))
    _w = (lambda a: (lambda t: t.astype(jnp.bfloat16) if jnp.issubdtype(t.dtype, jnp.floating) else t)(jnp.asarray(a)))
    B, S, D, H = 1, 2048, 1024, 32
    Dh = D // H
    return {
        "x": _w((lambda *s: _rng.normal(s) * 0.4)(B, S, D)),
        "wqkv": _w((lambda *s: _rng.normal(s) * 0.4)(D, 3 * D)),
        "w_phi": _w((lambda *s: _rng.normal(s) * 0.4)(H, Dh, Dh) * (Dh ** -0.5)),
        "wo": _w((lambda *s: _rng.normal(s) * 0.05)(D, D)),
    }

def reference(x, wqkv, w_phi, wo):
    B, S, D = x.shape
    H = 32; Dh = D // H
    qkv = (lambda x, *d: x.transpose(*d))((x @ wqkv).reshape(B, S, 3, H, Dh), 2, 0, 3, 1, 4)
    q, k, v = qkv[0], qkv[1], qkv[2]
    pq = jnp.einsum("bhsd,hdf->bhsf", q, w_phi)
    pk = jnp.einsum("bhsd,hdf->bhsf", k, w_phi)
    phi_q = jnp.concatenate([_softmax(pq, axis=-1), _softmax(-pq, axis=-1)], axis=-1)
    phi_k = jnp.concatenate([_softmax(pk, axis=-1), _softmax(-pk, axis=-1)], axis=-1)
    kv = jnp.einsum("bhsf,bhsd->bhfd", phi_k, v)
    z  = jnp.einsum("bhsf->bhf", phi_k)
    num = jnp.einsum("bhqf,bhfd->bhqd", phi_q, kv)
    den = jnp.einsum("bhqf,bhf->bhq", phi_q, z)[..., None] + 1e-6
    o = num / den
    return (lambda x, *d: x.transpose(*d))(o, 0, 2, 1, 3).reshape(B, S, D) @ wo
```

```python
import functools
import jax
import jax.numpy as jnp
from jax import lax
import jax.experimental.pallas as pl
import jax.experimental.pallas.tpu as pltpu

S, D, H, DH = 2048, 1024, 32, 32
G = D // 128
T = 512
NT = S // T
F32 = jnp.float32
BF16 = jnp.bfloat16


def _dual_softmax(s):
    s3 = s.reshape(4, DH, T)
    mx = jnp.max(s3, axis=1, keepdims=True)
    mn = jnp.min(s3, axis=1, keepdims=True)
    ep = jnp.exp(s3 - mx)
    en = jnp.exp(mn - s3)
    rp = 1.0 / jnp.sum(ep, axis=1, keepdims=True)
    rn = 1.0 / jnp.sum(en, axis=1, keepdims=True)
    return (ep * rp).reshape(128, T), (en * rn).reshape(128, T)


def _kernel(x_ref, wqkv_ref, wphi_ref, wo_ref, o_ref,
            wT, kv_acc, z_acc, lhs2, oT):
    p = pl.program_id(0)
    i = pl.program_id(1)

    @pl.when(jnp.logical_and(p == 0, i == 0))
    def _init():
        row = lax.broadcasted_iota(jnp.int32, (128, 128), 0) // DH
        col = lax.broadcasted_iota(jnp.int32, (128, 128), 1) // DH
        diag = row == col
        for g in range(G):
            w4 = wphi_ref[g * 128:(g + 1) * 128, :].astype(F32)
            w4 = jnp.concatenate([w4, w4, w4, w4], axis=1)
            at = jnp.where(diag, w4, 0.0)
            a = at.T.astype(BF16)
            for c in range(2):
                wg = wqkv_ref[:, c * D + g * 128: c * D + (g + 1) * 128]
                r = lax.dot_general(a, wg, (((1,), (1,)), ((), ())),
                                    preferred_element_type=F32)
                wT[c * D + g * 128: c * D + (g + 1) * 128, :] = r.astype(BF16)
        kv_acc[...] = jnp.zeros_like(kv_acc)
        z_acc[...] = jnp.zeros_like(z_acc)

    x = x_ref[...]

    @pl.when(p == 0)
    def _phase1():
        v = jnp.dot(x, wqkv_ref[:, 2 * D:], preferred_element_type=F32).astype(BF16)
        for g in range(G):
            kT = lax.dot_general(wT[D + g * 128: D + (g + 1) * 128, :], x,
                                 (((1,), (1,)), ((), ())), preferred_element_type=F32)
            pp, pn = _dual_softmax(kT)
            ppb = pp.astype(BF16)
            pnb = pn.astype(BF16)
            vg = v[:, g * 128:(g + 1) * 128]
            kv_acc[2 * g] += jnp.dot(ppb, vg, preferred_element_type=F32)
            kv_acc[2 * g + 1] += jnp.dot(pnb, vg, preferred_element_type=F32)
            ppf = ppb.astype(F32)
            pnf = pnb.astype(F32)
            zp = ppf[:, 0:128]
            zn = pnf[:, 0:128]
            for c in range(1, T // 128):
                zp = zp + ppf[:, c * 128:(c + 1) * 128]
                zn = zn + pnf[:, c * 128:(c + 1) * 128]
            z_acc[2 * g] += zp
            z_acc[2 * g + 1] += zn

    @pl.when(jnp.logical_and(p == 0, i == NT - 1))
    def _transition():
        row = lax.broadcasted_iota(jnp.int32, (128, 128), 0) // DH
        col = lax.broadcasted_iota(jnp.int32, (128, 128), 1) // DH
        diag = row == col
        zrow = lax.broadcasted_iota(jnp.int32, (16, 128), 0)
        zcol = lax.broadcasted_iota(jnp.int32, (16, 128), 1) // DH
        zdiag = zrow == zcol
        for g in range(G):
            for c in range(2):
                kvt = jnp.where(diag, kv_acc[2 * g + c].T, 0.0)
                lhs2[g, 0:128, c * 128:(c + 1) * 128] = kvt.astype(BF16)
                zr = jnp.sum(z_acc[2 * g + c].T, axis=0, keepdims=True)
                zr = jnp.where(zdiag, jnp.broadcast_to(zr, (16, 128)), 0.0)
                lhs2[g, 128:144, c * 128:(c + 1) * 128] = zr.astype(BF16)

    @pl.when(p == 1)
    def _phase2():
        for g in range(G):
            qT = lax.dot_general(wT[g * 128:(g + 1) * 128, :], x,
                                 (((1,), (1,)), ((), ())), preferred_element_type=F32)
            pp, pn = _dual_softmax(qT)
            phi = jnp.concatenate([pp.astype(BF16), pn.astype(BF16)], axis=0)
            nd = jnp.dot(lhs2[g], phi, preferred_element_type=F32)
            num = nd[0:128].reshape(4, DH, T)
            den = nd[128:136][0:4].reshape(4, 1, T) + 1e-6
            o = num / den
            oT[g * 128:(g + 1) * 128, :] = o.reshape(128, T).astype(BF16)
        out = lax.dot_general(oT[...], wo_ref[...], (((0,), (0,)), ((), ())),
                              preferred_element_type=F32)
        o_ref[...] = out.astype(o_ref.dtype)


@jax.jit
def pallas_standalone__linear_kernel_hedgehog__prompt_kernel(x, wqkv, w_phi, wo):
    x2 = x.reshape(S, D)
    wphi2 = w_phi.reshape(H * DH, DH)
    out = pl.pallas_call(
        _kernel,
        grid=(2, NT),
        in_specs=[
            pl.BlockSpec((T, D), lambda p, i: (i, 0)),
            pl.BlockSpec((D, 3 * D), lambda p, i: (0, 0)),
            pl.BlockSpec((H * DH, DH), lambda p, i: (0, 0)),
            pl.BlockSpec((D, D), lambda p, i: (0, 0)),
        ],
        out_specs=pl.BlockSpec((T, D), lambda p, i: (i * p, 0)),
        out_shape=jax.ShapeDtypeStruct((S, D), x.dtype),
        scratch_shapes=[
            pltpu.VMEM((2 * D, D), BF16),
            pltpu.VMEM((2 * G, 128, 128), F32),
            pltpu.VMEM((2 * G, 128, 128), F32),
            pltpu.VMEM((G, 144, 256), BF16),
            pltpu.VMEM((D, T), BF16),
        ],
        compiler_params=pltpu.CompilerParams(
            dimension_semantics=("arbitrary", "arbitrary"),
            vmem_limit_bytes=100 * 1024 * 1024,
        ),
    )(x2, wqkv, wphi2, wo)
    return out.reshape(1, S, D)
```

```python
import jax
import jax.numpy as jnp
from jax import lax
import jax.experimental.pallas as pl
import jax.experimental.pallas.tpu as pltpu

S, D, H, DH = 2048, 1024, 32, 32
G = D // 128
T = 512
TH = T // 2
NT = S // T
VC = 4
CW = D // VC
EC = 8
ER = T // EC
F32 = jnp.float32
BF16 = jnp.bfloat16

SEM_X = 0
SEM_WV = SEM_X + NT
SEM_WQK = SEM_WV + VC
SEM_WO = SEM_WQK + 2
SEM_OUT = SEM_WO + 1
SEM_EP = SEM_OUT + 2
SEM_WPHI = SEM_EP + EC
SEM_X0 = SEM_WPHI + 1
NSEM = SEM_X0 + 2

_NT = (((1,), (1,)), ((), ()))


def _dual_softmax(s):
    s3 = s.reshape(4, DH, T)
    mx = jnp.max(s3, axis=1, keepdims=True)
    mn = jnp.min(s3, axis=1, keepdims=True)
    ep = jnp.exp(s3 - mx)
    en = jnp.exp(mn - s3)
    rp = 1.0 / jnp.sum(ep, axis=1, keepdims=True)
    rn = 1.0 / jnp.sum(en, axis=1, keepdims=True)
    return (ep * rp).reshape(128, T), (en * rn).reshape(128, T)


def _kernel(x_hbm, wqkv_hbm, wphi_hbm, wo_hbm, o_hbm,
            xv, wraw, wv, wo_v, wT, kv_acc, z_acc, lhs2, on, obuf, v0, wphi_ref, ablk, vacc, sems):

    def x_copy(c):
        return pltpu.make_async_copy(x_hbm.at[pl.ds(c * T, T), :], xv.at[c], sems.at[SEM_X + c])

    def x0_copy(hf):
        return pltpu.make_async_copy(x_hbm.at[hf * TH:(hf + 1) * TH, :],
                                     xv.at[0, hf * TH:(hf + 1) * TH, :], sems.at[SEM_X0 + hf])

    def wv_copy(c):
        return pltpu.make_async_copy(wqkv_hbm.at[c * CW:(c + 1) * CW, 2 * D:3 * D],
                                     wv.at[c * CW:(c + 1) * CW, :], sems.at[SEM_WV + c])

    def wqk_copy(c):
        return pltpu.make_async_copy(wqkv_hbm.at[:, c * D:(c + 1) * D], wraw.at[c], sems.at[SEM_WQK + c])

    def wphi_copy():
        return pltpu.make_async_copy(wphi_hbm, wphi_ref, sems.at[SEM_WPHI])

    def wo_copy():
        return pltpu.make_async_copy(wo_hbm, wo_v, sems.at[SEM_WO])

    def out_copy(i, slot):
        return pltpu.make_async_copy(obuf.at[slot], o_hbm.at[pl.ds(i * T, T), :], sems.at[SEM_OUT + slot])

    def ep_copy(c, slot):
        return pltpu.make_async_copy(obuf.at[slot, pl.ds(c * ER, ER), :],
                                     o_hbm.at[pl.ds((NT - 1) * T + c * ER, ER), :], sems.at[SEM_EP + c])

    row = lax.broadcasted_iota(jnp.int32, (128, 128), 0) // DH
    col = lax.broadcasted_iota(jnp.int32, (128, 128), 1) // DH
    diag = row == col

    def fold(c):
        for g in range(G):
            r = lax.dot_general(ablk[g], wraw[c, :, g * 128:(g + 1) * 128], _NT,
                                preferred_element_type=F32)
            wT[c * D + g * 128: c * D + (g + 1) * 128, :] = r.astype(BF16)

    def phase1_tile(i, first):
        x = xv[i]
        kT = lax.dot_general(wT[D:2 * D, :], x, _NT, preferred_element_type=F32)
        if first:
            vb = v0[...]
        else:
            vb = jnp.dot(x, wv[...], preferred_element_type=F32).astype(BF16)
        for g in range(G):
            pp, pn = _dual_softmax(kT[g * 128:(g + 1) * 128])
            phi = jnp.concatenate([pp.astype(BF16), pn.astype(BF16)], axis=0)
            kv_acc[g] += jnp.dot(phi, vb[:, g * 128:(g + 1) * 128], preferred_element_type=F32)
            pf = phi.astype(F32)
            zz = pf[:, 0:128]
            for c in range(1, T // 128):
                zz = zz + pf[:, c * 128:(c + 1) * 128]
            z_acc[g] += zz

    wphi_copy().start()
    x0_copy(0).start()
    wv_copy(0).start()
    x0_copy(1).start()
    for c in range(1, VC):
        wv_copy(c).start()
    wqk_copy(1).start()
    for c in range(1, NT):
        x_copy(c).start()
    kv_acc[...] = jnp.zeros_like(kv_acc)
    z_acc[...] = jnp.zeros_like(z_acc)

    wphi_copy().wait()
    for g in range(G):
        w4 = wphi_ref[g * 128:(g + 1) * 128, :].astype(F32)
        w4 = jnp.concatenate([w4, w4, w4, w4], axis=1)
        ablk[g] = jnp.where(diag, w4, 0.0).T.astype(BF16)

    x0_copy(0).wait()
    wv_copy(0).wait()
    vacc[0:TH, :] = jnp.dot(xv[0, 0:TH, 0:CW], wv[0:CW, :], preferred_element_type=F32)
    x0_copy(1).wait()
    vacc[TH:T, :] = jnp.dot(xv[0, TH:T, 0:CW], wv[0:CW, :], preferred_element_type=F32)
    for c in range(1, VC):
        wv_copy(c).wait()
        part = vacc[...] + jnp.dot(xv[0, :, c * CW:(c + 1) * CW], wv[c * CW:(c + 1) * CW, :],
                                   preferred_element_type=F32)
        if c + 1 < VC:
            vacc[...] = part
        else:
            v0[...] = part.astype(BF16)
    wqk_copy(1).wait()
    wqk_copy(0).start()
    wo_copy().start()
    fold(1)
    phase1_tile(0, True)

    def p1_body(i, carry):
        x_copy(i).wait()
        phase1_tile(i, False)
        return carry
    lax.fori_loop(1, NT, p1_body, 0)

    wqk_copy(0).wait()
    wo_copy().wait()
    fold(0)
    for g in range(G):
        for c in range(2):
            kvt = jnp.where(diag, kv_acc[g, c * 128:(c + 1) * 128, :].T, 0.0)
            lhs2[g, :, c * 128:(c + 1) * 128] = kvt.astype(BF16)
        zs = jnp.sum(z_acc[g], axis=1, keepdims=True)
        z_acc[g] = jnp.broadcast_to(zs, (256, 128))

    def phase2_tile(i, do_out):
        x = xv[i]
        cur = i % 2
        qT = lax.dot_general(wT[0:D, :], x, _NT, preferred_element_type=F32)
        if do_out:
            prev = (i - 1) % 2
            obuf[prev] = jnp.dot(on[prev], wo_v[...], preferred_element_type=F32).astype(BF16)
        for g in range(G):
            pp, pn = _dual_softmax(qT[g * 128:(g + 1) * 128])
            phi = jnp.concatenate([pp.astype(BF16), pn.astype(BF16)], axis=0)
            num = jnp.dot(lhs2[g], phi, preferred_element_type=F32).reshape(4, DH, T)
            zp = z_acc[g, 0:128, :]
            zn = z_acc[g, 128:256, :]
            zp = jnp.concatenate([zp] * (T // 128), axis=1)
            zn = jnp.concatenate([zn] * (T // 128), axis=1)
            den = jnp.sum((pp * zp + pn * zn).reshape(4, DH, T), axis=1, keepdims=True) + 1e-6
            o = (num * (1.0 / den)).reshape(128, T)
            on[cur, :, g * 128:(g + 1) * 128] = o.T.astype(BF16)
        if do_out:
            out_copy(i - 1, prev).start()

    phase2_tile(0, False)

    def p2_body(i, carry):
        @pl.when(i >= 3)
        def _():
            out_copy(i - 3, (i - 1) % 2).wait()
        phase2_tile(i, True)
        return carry
    lax.fori_loop(1, NT, p2_body, 0)

    last = (NT - 1) % 2
    out_copy(NT - 3, last).wait()
    for c in range(EC):
        obuf[last, c * ER:(c + 1) * ER, :] = jnp.dot(on[last, c * ER:(c + 1) * ER, :], wo_v[...],
                                                    preferred_element_type=F32).astype(BF16)
        ep_copy(c, last).start()
    out_copy(NT - 2, (NT - 2) % 2).wait()
    for c in range(EC):
        ep_copy(c, last).wait()


@jax.jit
def pallas_standalone__linear_kernel_hedgehog__prompt_kernel(x, wqkv, w_phi, wo):
    x2 = x.reshape(S, D)
    wphi2 = w_phi.reshape(H * DH, DH)
    out = pl.pallas_call(
        _kernel,
        in_specs=[
            pl.BlockSpec(memory_space=pl.ANY),
            pl.BlockSpec(memory_space=pl.ANY),
            pl.BlockSpec(memory_space=pl.ANY),
            pl.BlockSpec(memory_space=pl.ANY),
        ],
        out_specs=pl.BlockSpec(memory_space=pl.ANY),
        out_shape=jax.ShapeDtypeStruct((S, D), x.dtype),
        scratch_shapes=[
            pltpu.VMEM((NT, T, D), BF16),
            pltpu.VMEM((2, D, D), BF16),
            pltpu.VMEM((D, D), BF16),
            pltpu.VMEM((D, D), BF16),
            pltpu.VMEM((2 * D, D), BF16),
            pltpu.VMEM((G, 256, 128), F32),
            pltpu.VMEM((G, 256, 128), F32),
            pltpu.VMEM((G, 128, 256), BF16),
            pltpu.VMEM((2, T, D), BF16),
            pltpu.VMEM((2, T, D), BF16),
            pltpu.VMEM((T, D), BF16),
            pltpu.VMEM((H * DH, DH), BF16),
            pltpu.VMEM((G, 128, 128), BF16),
            pltpu.VMEM((T, D), F32),
            pltpu.SemaphoreType.DMA((NSEM,)),
        ],
        compiler_params=pltpu.CompilerParams(
            vmem_limit_bytes=100 * 1024 * 1024,
        ),
    )(x2, wqkv, wphi2, wo)
    return out.reshape(1, S, D)
```
